```python
import os as _os
_os.environ.setdefault("JAX_PLATFORMS", "cpu")
import jax
import jax.numpy as jnp

def _softmax(x, axis=-1):
    return jax.nn.softmax(x, axis=axis)
def _gelu(x):
    return jax.nn.gelu(x, approximate=True)
def _silu(x):
    return jax.nn.silu(x)
def _sigmoid(x):
    return jax.nn.sigmoid(x)
def _layernorm(x, axis=-1, eps=1e-5):
    m = jnp.mean(x, axis=axis, keepdims=True)
    v = jnp.var(x, axis=axis, keepdims=True)
    return (x - m) / jnp.sqrt(v + eps)
def _scatter_add(tgt, idx, src, axis=0):
    return tgt.at[idx].add(src)
def _segment_sum(src, seg, n):
    return jax.ops.segment_sum(src, seg, n)
class _Rng:
    def __init__(self, key):
        self._k = key
    def _next(self):
        self._k, sub = jax.random.split(self._k)
        return sub
    def normal(self, shape):
        return jax.random.normal(self._next(), shape, dtype=jnp.bfloat16)
    def randint(self, lo, hi, shape):
        return jax.random.randint(self._next(), shape, lo, hi, dtype=jnp.int32)
    def uniform(self, shape, lo=0.0, hi=1.0):
        return jax.random.uniform(self._next(), shape, jnp.bfloat16, lo, hi)
    def permutation(self, n):
        return jax.random.permutation(self._next(), n)


kernel_name = 'gated_mix__sliding_block_cached__dense_activation_silu__decode'

def setup_inputs():
    _rng = _Rng(jax.random.key(int.from_bytes(__import__("os").urandom(4), "little")))
    _w = (lambda a: (lambda t: t.astype(jnp.bfloat16) if jnp.issubdtype(t.dtype, jnp.floating) else t)(jnp.asarray(a)))
    def _A_setup():
        B, Sq, D = 2, 1, 1024
        Hq, Hkv, Sk, Dh = 32, 4, 32768, 128
        assert Hq % Hkv == 0, (Hq, Hkv)
        return {
            "x": _w((lambda *s: _rng.normal(s) * 0.05)(B, Sq, D)),
            "k_cache": _w((lambda *s: _rng.normal(s) * 3.2)(B, Hkv, Sk, Dh)),
            "v_cache": _w((lambda *s: _rng.normal(s) * 0.05)(B, Hkv, Sk, Dh)),
            "wq": _w((lambda *s: _rng.normal(s) * 3.2)(D, Hq * Dh) * (D ** -0.5)),
            "wo": _w((lambda *s: _rng.normal(s) * 0.05)(Hq * Dh, D) * ((Hq * Dh) ** -0.5)),
        }
    _A_in = _A_setup()

    def _B_setup():
        B, S, D, F = 2, 1, 1024, 3584
        return {
            "x": _w((lambda *s: _rng.normal(s) * 0.05)(B, S, D)),
            "w1": _w((lambda *s: _rng.normal(s) * 0.05)(D, F) * (D ** -0.5)),
            "w2": _w((lambda *s: _rng.normal(s) * 0.05)(F, D) * (F ** -0.5)),
        }
    _B_in = _B_setup()

    return {
        "A_x": _A_in["x"],
        "A_k_cache": _A_in["k_cache"],
        "A_v_cache": _A_in["v_cache"],
        "A_wq": _A_in["wq"],
        "A_wo": _A_in["wo"],
        "B_x": _B_in["x"],
        "B_w1": _B_in["w1"],
        "B_w2": _B_in["w2"],
        "gate_w": _w((lambda *s: _rng.normal(s) * 0.05)(1024) * 16.0),
    }

def reference(A_x, A_k_cache, A_v_cache, A_wq, A_wo, B_x, B_w1, B_w2, gate_w):
    def _A_ref(x, k_cache, v_cache, wq, wo):
        B, Sq, D = x.shape
        Hq, Dh = 32, 128
        Hkv, Sk = k_cache.shape[1], k_cache.shape[2]
        W = min(4096, max(256, Sk // 4))
        rep = Hq // Hkv
        q = (lambda x, *d: x.transpose(*d))((x @ wq).reshape(B, Sq, Hq, Dh), 0, 2, 1, 3)
        k = jnp.repeat(k_cache[:, :, Sk - W:, :], rep, axis=1)
        v = jnp.repeat(v_cache[:, :, Sk - W:, :], rep, axis=1)
        scores = jnp.einsum("bhqd,bhkd->bhqk", q, k) * (Dh ** -0.5)
        p = _softmax(scores, axis=-1)
        o = jnp.einsum("bhqk,bhkd->bhqd", p, v)
        return (lambda x, *d: x.transpose(*d))(o, 0, 2, 1, 3).reshape(B, Sq, Hq * Dh) @ wo

    def _B_ref(x, w1, w2):
        h = jnp.einsum("bsd,df->bsf", x, w1)
        h = _silu(h)
        out = jnp.einsum("bsf,fd->bsd", h, w2)
        return out

    x = A_x
    g = _sigmoid((x * gate_w).sum(-1, keepdims=True))
    a = _A_ref(x, A_k_cache, A_v_cache, A_wq, A_wo)
    b = _B_ref(x, B_w1, B_w2)
    return g * a + (1 - g) * b
```

```python
import jax
import jax.numpy as jnp
import jax.experimental.pallas as pl
import jax.experimental.pallas.tpu as pltpu

HQ, DH = 32, 128


def make(wq_c=8, w1_c=4, wo_c=4, w2_c=14, compute=True):
    def fn(A_x, A_k_cache, A_v_cache, A_wq, A_wo, B_x, B_w1, B_w2, gate_w):
        B, Sq, D = A_x.shape
        _, HKV, Sk, _ = A_k_cache.shape
        W = min(4096, max(256, Sk // 4))
        REP = HQ // HKV
        F = B_w1.shape[1]
        assert B == 2 and Sq == 1 and REP == 8

        def kernel(x_h, k_h, v_h, wq_h, wo_h, w1_h, w2_h, g_h, o_ref,
                   x_v, g_v, k_v, v_v, wq_v, wo_v, w1_v, w2_v, sems):
            cps = {}
            n = [0]
            def add(name, src, dst):
                c = pltpu.make_async_copy(src, dst, sems.at[n[0]])
                n[0] += 1
                c.start()
                cps[name] = c
            add('x', x_h, x_v)
            rq = D // wq_c
            for i in range(wq_c):
                add(('wq', i), wq_h.at[pl.ds(i * rq, rq)], wq_v.at[pl.ds(i * rq, rq)])
            add('g', g_h, g_v)
            for g in range(HKV):
                for b in range(B):
                    add(('k', b, g), k_h.at[b, g, pl.ds(Sk - W, W)], k_v.at[b, g])
                    add(('v', b, g), v_h.at[b, g, pl.ds(Sk - W, W)], v_v.at[b, g])
            r1 = D // w1_c
            for i in range(w1_c):
                add(('w1', i), w1_h.at[pl.ds(i * r1, r1)], w1_v.at[pl.ds(i * r1, r1)])
            ro = HQ * DH // wo_c
            for i in range(wo_c):
                add(('wo', i), wo_h.at[pl.ds(i * ro, ro)], wo_v.at[pl.ds(i * ro, ro)])
            r2 = F // w2_c
            for i in range(w2_c):
                add(('w2', i), w2_h.at[pl.ds(i * r2, r2)], w2_v.at[pl.ds(i * r2, r2)])

            if not compute:
                for c in cps.values():
                    c.wait()
                o_ref[...] = x_v[...]
                return

            cps['x'].wait()
            row = jax.lax.broadcasted_iota(jnp.int32, (16, D), 0)
            x0 = jnp.broadcast_to(x_v[0:1].astype(jnp.float32), (16, D))
            x1 = jnp.broadcast_to(x_v[1:2].astype(jnp.float32), (16, D))
            xf = jnp.where(row < 8, x0, x1)
            x16 = xf.astype(jnp.bfloat16)
            q = jnp.zeros((16, HQ * DH), jnp.float32)
            for i in range(wq_c):
                cps[('wq', i)].wait()
                q += jnp.dot(x16[:, i * rq:(i + 1) * rq], wq_v[pl.ds(i * rq, rq), :],
                             preferred_element_type=jnp.float32)
            cps['g'].wait()
            gw = g_v[...].astype(jnp.float32).reshape(1, D)
            gate = jax.nn.sigmoid(jnp.sum(xf * gw, axis=-1, keepdims=True))
            r8 = jax.lax.broadcasted_iota(jnp.int32, (8, DH), 0)
            r16 = jax.lax.broadcasted_iota(jnp.int32, (16, DH), 0) % 8
            scale = DH ** -0.5
            lhs = []
            for g in range(HKV):
                os_ = []
                for b in range(B):
                    qg = jnp.zeros((8, DH), jnp.float32)
                    for r in range(REP):
                        h = g * REP + r
                        qg = jnp.where(r8 == r, q[b * 8:(b + 1) * 8, h * DH:(h + 1) * DH], qg)
                    cps[('k', b, g)].wait()
                    s = jax.lax.dot_general(qg.astype(jnp.bfloat16), k_v[b, g],
                                            (((1,), (1,)), ((), ())),
                                            preferred_element_type=jnp.float32) * scale
                    m = jnp.max(s, axis=-1, keepdims=True)
                    p = jnp.exp(s - m)
                    l = jnp.sum(p, axis=-1, keepdims=True)
                    cps[('v', b, g)].wait()
                    o = jnp.dot(p.astype(jnp.bfloat16), v_v[b, g], preferred_element_type=jnp.float32)
                    os_.append(o / l)
                og = jnp.concatenate(os_, axis=0)
                for r in range(REP):
                    lhs.append(jnp.where(r16 == r, og, 0.0).astype(jnp.bfloat16))
            ol = jnp.concatenate(lhs, axis=1)
            h1 = jnp.zeros((16, F), jnp.float32)
            for i in range(w1_c):
                cps[('w1', i)].wait()
                h1 += jnp.dot(x16[:, i * r1:(i + 1) * r1], w1_v[pl.ds(i * r1, r1), :],
                              preferred_element_type=jnp.float32)
            hb = (h1 * jax.nn.sigmoid(h1)).astype(jnp.bfloat16)
            a = jnp.zeros((16, D), jnp.float32)
            for i in range(wo_c):
                cps[('wo', i)].wait()
                a += jnp.dot(ol[:, i * ro:(i + 1) * ro], wo_v[pl.ds(i * ro, ro), :],
                             preferred_element_type=jnp.float32)
            bo = jnp.zeros((16, D), jnp.float32)
            for i in range(w2_c):
                cps[('w2', i)].wait()
                bo += jnp.dot(hb[:, i * r2:(i + 1) * r2], w2_v[pl.ds(i * r2, r2), :],
                              preferred_element_type=jnp.float32)
            tot = gate * a + jnp.where(row % 8 == 0, (1.0 - gate) * bo, 0.0)
            for b in range(B):
                o_ref[b:b+1] = jnp.sum(tot[b * 8:(b + 1) * 8], axis=0, keepdims=True).astype(o_ref.dtype)

        nsem = 2 + wq_c + 2 * B * HKV + w1_c + wo_c + w2_c
        anyspec = pl.BlockSpec(memory_space=pl.ANY)
        bf = jnp.bfloat16
        return pl.pallas_call(
            kernel,
            out_shape=jax.ShapeDtypeStruct((B, D), A_x.dtype),
            in_specs=[anyspec] * 8,
            out_specs=pl.BlockSpec(memory_space=pltpu.VMEM),
            scratch_shapes=[
                pltpu.VMEM((B, D), bf), pltpu.VMEM((D,), bf),
                pltpu.VMEM((B, HKV, W, DH), bf), pltpu.VMEM((B, HKV, W, DH), bf),
                pltpu.VMEM(A_wq.shape, bf), pltpu.VMEM(A_wo.shape, bf),
                pltpu.VMEM(B_w1.shape, bf), pltpu.VMEM(B_w2.shape, bf),
                pltpu.SemaphoreType.DMA((nsem,)),
            ],
            compiler_params=pltpu.CompilerParams(vmem_limit_bytes=100 * 1024 * 1024),
        )(A_x.reshape(B, D), A_k_cache, A_v_cache, A_wq, A_wo, B_w1, B_w2, gate_w).reshape(B, Sq, D)
    return jax.jit(fn)


pallas_gated_mix__sliding_block_cached__dense_activation_silu__decode_kernel = make()
```

```python
import jax
import jax.numpy as jnp
import jax.experimental.pallas as pl
import jax.experimental.pallas.tpu as pltpu

HQ, DH = 32, 128


def make(wq_c=1, w1_c=1, wo_c=2, w2s=(512,) * 6 + (256, 128, 128)):
    def fn(A_x, A_k_cache, A_v_cache, A_wq, A_wo, B_x, B_w1, B_w2, gate_w):
        B, Sq, D = A_x.shape
        _, HKV, Sk, _ = A_k_cache.shape
        W = min(4096, max(256, Sk // 4))
        REP = HQ // HKV
        F = B_w1.shape[1]
        assert B == 2 and Sq == 1 and REP == 8

        off = [sum(w2s[:i]) for i in range(len(w2s))]
        assert sum(w2s) == F
        def kernel(x_h, k_h, v_h, wq_h, wo_h, w1_h, w2_h, g_h, o_ref,
                   x_v, g_v, k_v, v_v, wq_v, wo_v, w1_v, w2_v, sems):
            cps = {}
            n = [0]
            def add(name, src, dst):
                c = pltpu.make_async_copy(src, dst, sems.at[n[0]])
                n[0] += 1
                c.start()
                cps[name] = c
            add('x', x_h, x_v)
            rq = D // wq_c
            for i in range(wq_c):
                add(('wq', i), wq_h.at[pl.ds(i * rq, rq)], wq_v.at[pl.ds(i * rq, rq)])
            add('g', g_h, g_v)
            add('k', k_h.at[:, :, pl.ds(Sk - W, W)], k_v)
            add('v', v_h.at[:, :, pl.ds(Sk - W, W)], v_v)
            r1 = D // w1_c
            for i in range(w1_c):
                add(('w1', i), w1_h.at[pl.ds(i * r1, r1)], w1_v.at[pl.ds(i * r1, r1)])
            ro = HQ * DH // wo_c
            for i in range(wo_c):
                add(('wo', i), wo_h.at[pl.ds(i * ro, ro)], wo_v.at[pl.ds(i * ro, ro)])
            for i in range(len(w2s)):
                add(('w2', i), w2_h.at[pl.ds(off[i], w2s[i])], w2_v.at[pl.ds(off[i], w2s[i])])

            cps['x'].wait()
            row = jax.lax.broadcasted_iota(jnp.int32, (16, D), 0)
            x0 = jnp.broadcast_to(x_v[0:1].astype(jnp.float32), (16, D))
            x1 = jnp.broadcast_to(x_v[1:2].astype(jnp.float32), (16, D))
            xf = jnp.where(row < 8, x0, x1)
            x16 = xf.astype(jnp.bfloat16)
            q = jnp.zeros((16, HQ * DH), jnp.float32)
            for i in range(wq_c):
                cps[('wq', i)].wait()
                q += jnp.dot(x16[:, i * rq:(i + 1) * rq], wq_v[pl.ds(i * rq, rq), :],
                             preferred_element_type=jnp.float32)
            cps['g'].wait()
            gw = g_v[...].astype(jnp.float32).reshape(1, D)
            gate = jax.nn.sigmoid(jnp.sum(xf * gw, axis=-1, keepdims=True))
            r8 = jax.lax.broadcasted_iota(jnp.int32, (8, DH), 0)
            r16 = jax.lax.broadcasted_iota(jnp.int32, (16, DH), 0) % 8
            scale = DH ** -0.5
            lhs = []
            cps['k'].wait()
            cps['v'].wait()
            for g in range(HKV):
                os_ = []
                for b in range(B):
                    qg = jnp.zeros((8, DH), jnp.float32)
                    for r in range(REP):
                        h = g * REP + r
                        qg = jnp.where(r8 == r, q[b * 8:(b + 1) * 8, h * DH:(h + 1) * DH], qg)
                    s = jax.lax.dot_general(qg.astype(jnp.bfloat16), k_v[b, g],
                                            (((1,), (1,)), ((), ())),
                                            preferred_element_type=jnp.float32) * scale
                    m = jnp.max(s, axis=-1, keepdims=True)
                    p = jnp.exp(s - m)
                    l = jnp.sum(p, axis=-1, keepdims=True)
                    o = jnp.dot(p.astype(jnp.bfloat16), v_v[b, g], preferred_element_type=jnp.float32)
                    os_.append(o / l)
                og = jnp.concatenate(os_, axis=0)
                for r in range(REP):
                    lhs.append(jnp.where(r16 == r, og, 0.0).astype(jnp.bfloat16))
            ol = jnp.concatenate(lhs, axis=1)
            h1 = jnp.zeros((16, F), jnp.float32)
            for i in range(w1_c):
                cps[('w1', i)].wait()
                h1 += jnp.dot(x16[:, i * r1:(i + 1) * r1], w1_v[pl.ds(i * r1, r1), :],
                              preferred_element_type=jnp.float32)
            hb = (h1 * jax.nn.sigmoid(h1)).astype(jnp.bfloat16)
            a = jnp.zeros((16, D), jnp.float32)
            for i in range(wo_c):
                cps[('wo', i)].wait()
                a += jnp.dot(ol[:, i * ro:(i + 1) * ro], wo_v[pl.ds(i * ro, ro), :],
                             preferred_element_type=jnp.float32)
            bo = jnp.zeros((16, D), jnp.float32)
            for i in range(len(w2s)):
                cps[('w2', i)].wait()
                bo += jnp.dot(hb[:, off[i]:off[i] + w2s[i]], w2_v[pl.ds(off[i], w2s[i]), :],
                              preferred_element_type=jnp.float32)
            tot = gate * a + jnp.where(row % 8 == 0, (1.0 - gate) * bo, 0.0)
            for b in range(B):
                o_ref[b:b+1] = jnp.sum(tot[b * 8:(b + 1) * 8], axis=0, keepdims=True).astype(o_ref.dtype)

        nsem = 2 + wq_c + 2 + w1_c + wo_c + len(w2s)
        anyspec = pl.BlockSpec(memory_space=pl.ANY)
        bf = jnp.bfloat16
        return pl.pallas_call(
            kernel,
            out_shape=jax.ShapeDtypeStruct((B, D), A_x.dtype),
            in_specs=[anyspec] * 8,
            out_specs=pl.BlockSpec(memory_space=pltpu.VMEM),
            scratch_shapes=[
                pltpu.VMEM((B, D), bf), pltpu.VMEM((D,), bf),
                pltpu.VMEM((B, HKV, W, DH), bf), pltpu.VMEM((B, HKV, W, DH), bf),
                pltpu.VMEM(A_wq.shape, bf), pltpu.VMEM(A_wo.shape, bf),
                pltpu.VMEM(B_w1.shape, bf), pltpu.VMEM(B_w2.shape, bf),
                pltpu.SemaphoreType.DMA((nsem,)),
            ],
            compiler_params=pltpu.CompilerParams(vmem_limit_bytes=100 * 1024 * 1024),
        )(A_x.reshape(B, D), A_k_cache, A_v_cache, A_wq, A_wo, B_w1, B_w2, gate_w).reshape(B, Sq, D)
    return jax.jit(fn)


pallas_gated_mix__sliding_block_cached__dense_activation_silu__decode_kernel = make()
```
